```python
import os as _os
_os.environ.setdefault("JAX_PLATFORMS", "cpu")
import jax
import jax.numpy as jnp

def _softmax(x, axis=-1):
    return jax.nn.softmax(x, axis=axis)
def _gelu(x):
    return jax.nn.gelu(x, approximate=True)
def _silu(x):
    return jax.nn.silu(x)
def _sigmoid(x):
    return jax.nn.sigmoid(x)
def _layernorm(x, axis=-1, eps=1e-5):
    m = jnp.mean(x, axis=axis, keepdims=True)
    v = jnp.var(x, axis=axis, keepdims=True)
    return (x - m) / jnp.sqrt(v + eps)
def _scatter_add(tgt, idx, src, axis=0):
    return tgt.at[idx].add(src)
def _segment_sum(src, seg, n):
    return jax.ops.segment_sum(src, seg, n)
class _Rng:
    def __init__(self, key):
        self._k = key
    def _next(self):
        self._k, sub = jax.random.split(self._k)
        return sub
    def normal(self, shape):
        return jax.random.normal(self._next(), shape, dtype=jnp.bfloat16)
    def randint(self, lo, hi, shape):
        return jax.random.randint(self._next(), shape, lo, hi, dtype=jnp.int32)
    def uniform(self, shape, lo=0.0, hi=1.0):
        return jax.random.uniform(self._next(), shape, jnp.bfloat16, lo, hi)
    def permutation(self, n):
        return jax.random.permutation(self._next(), n)


kernel_name = 'interleave_layers__gqa_block_cached__dense_activation_mish__decode'

def setup_inputs():
    _rng = _Rng(jax.random.key(int.from_bytes(__import__("os").urandom(4), "little")))
    _w = (lambda a: (lambda t: t.astype(jnp.bfloat16) if jnp.issubdtype(t.dtype, jnp.floating) else t)(jnp.asarray(a)))
    def _A_setup():
        B, Sq, D = 1, 1, 512
        Hq, Hkv, Sk, Dh = 32, 8, 65536, 128
        assert Hq % Hkv == 0, (Hq, Hkv)
        return {
            "x": _w((lambda *s: _rng.normal(s) * 0.05)(B, Sq, D)),
            "k_cache": _w((lambda *s: _rng.normal(s) * 1.6)(B, Hkv, Sk, Dh)),
            "v_cache": _w((lambda *s: _rng.normal(s) * 1.6)(B, Hkv, Sk, Dh)),
            "wq": _w((lambda *s: _rng.normal(s) * 1.6)(D, Hq * Dh) * (D ** -0.5)),
            "wo": _w((lambda *s: _rng.normal(s) * 1.6)(Hq * Dh, D) * ((Hq * Dh) ** -0.5)),
        }
    _A_in = _A_setup()

    def _B_setup():
        B, S, D, F = 1, 1, 512, 1792
        return {
            "x": _w((lambda *s: _rng.normal(s) * 0.05)(B, S, D)),
            "w1": _w((lambda *s: _rng.normal(s) * 0.8)(D, F) * (D ** -0.5)),
            "b1": _w((lambda *s: _rng.normal(s) * 0.8)(F)),
            "w2": _w((lambda *s: _rng.normal(s) * 0.8)(F, D) * (F ** -0.5)),
        }
    _B_in = _B_setup()

    return {
        "A_x": _A_in["x"],
        "A_k_cache": _A_in["k_cache"],
        "A_v_cache": _A_in["v_cache"],
        "A_wq": _A_in["wq"],
        "A_wo": _A_in["wo"],
        "B_x": _B_in["x"],
        "B_w1": _B_in["w1"],
        "B_b1": _B_in["b1"],
        "B_w2": _B_in["w2"],
    }

def reference(A_x, A_k_cache, A_v_cache, A_wq, A_wo, B_x, B_w1, B_b1, B_w2):
    def _A_ref(x, k_cache, v_cache, wq, wo):
        B, Sq, D = x.shape
        Hq, Dh = 32, 128
        Hkv = k_cache.shape[1]
        rep = Hq // Hkv
        q = (lambda x, *d: x.transpose(*d))((x @ wq).reshape(B, Sq, Hq, Dh), 0, 2, 1, 3)
        k = jnp.repeat(k_cache, rep, axis=1)
        v = jnp.repeat(v_cache, rep, axis=1)
        scores = jnp.einsum("bhqd,bhkd->bhqk", q, k) * (Dh ** -0.5)
        p = _softmax(scores, axis=-1)
        o = jnp.einsum("bhqk,bhkd->bhqd", p, v)
        return (lambda x, *d: x.transpose(*d))(o, 0, 2, 1, 3).reshape(B, Sq, Hq * Dh) @ wo

    def _B_ref(x, w1, b1, w2):
        h = jnp.einsum("bsd,df->bsf", x, w1) + b1
        sp = jnp.log1p(jnp.exp(-jnp.abs(h))) + jnp.where(h > 0, h, jnp.zeros_like(h))
        act = h * jnp.tanh(sp)
        return jnp.einsum("bsf,fd->bsd", act, w2)

    x = A_x
    x = x + _A_ref(_layernorm(x, axis=-1), A_k_cache, A_v_cache, A_wq, A_wo)
    x = x + _B_ref(_layernorm(x, axis=-1), B_w1, B_b1, B_w2)
    x = x + _A_ref(_layernorm(x, axis=-1), A_k_cache, A_v_cache, A_wq, A_wo)
    x = x + _B_ref(_layernorm(x, axis=-1), B_w1, B_b1, B_w2)
    return x
```

```python
import jax
import jax.numpy as jnp
from jax import lax
import jax.experimental.pallas as pl
import jax.experimental.pallas.tpu as pltpu

D = 512
HQ = 32
HKV = 8
SK = 65536
DH = 128
F = 1792
REP = HQ // HKV
GW = REP * DH
EPS = 1e-5

A_ROWS = 1152
B_ROWS = 896
CHUNK = A_ROWS + B_ROWS
NSTEP = SK // CHUNK
T = HKV * NSTEP
NBUF = 4
NEXTRA = 3
EXTRA_PERIOD = 64
EXTRA_PHASE = 40
LOOK = NBUF - 1
VMEM_LIMIT = 128 * 1024 * 1024

_NT = (((1,), (1,)), ((), ()))


def _layernorm(x):
    m = jnp.mean(x, axis=-1, keepdims=True)
    xc = x - m
    v = jnp.mean(xc * xc, axis=-1, keepdims=True)
    return xc / jnp.sqrt(v + EPS)


def _kernel(x_ref, b1_ref, k_hbm, v_hbm, wq_hbm, wo_hbm, w1_hbm, w2_hbm, o_ref,
            kbuf, vbuf, kres, vres, wq_v, wo_v, w1_v, w2_v,
            sk, sv, srk, srv, swq, sw):
    f32 = jnp.float32
    bf16 = jnp.bfloat16
    scale = DH ** -0.5

    def is_extra(t):
        if NEXTRA == 0:
            return False
        return jnp.logical_and(t % EXTRA_PERIOD == EXTRA_PHASE, t < NEXTRA * EXTRA_PERIOD)

    def a_slot(g, t):
        if NEXTRA == 0:
            return g % NBUF
        return jnp.where(is_extra(t), NBUF + t // EXTRA_PERIOD, g % NBUF)

    def stream_copies(t, slot, sem):
        off = pl.multiple_of(t * CHUNK, 128)
        return (
            pltpu.make_async_copy(k_hbm.at[pl.ds(off, A_ROWS)], kbuf.at[slot], sk.at[sem]),
            pltpu.make_async_copy(v_hbm.at[pl.ds(off, A_ROWS)], vbuf.at[slot], sv.at[sem]),
        )

    def res_copies(t, sem):
        off = pl.multiple_of(t * CHUNK + A_ROWS, 128)
        return (
            pltpu.make_async_copy(k_hbm.at[pl.ds(off, B_ROWS)], kres.at[t], srk.at[sem]),
            pltpu.make_async_copy(v_hbm.at[pl.ds(off, B_ROWS)], vres.at[t], srv.at[sem]),
        )

    def wq_copy(h):
        off = h * GW if isinstance(h, int) else pl.multiple_of(h * GW, GW)
        return pltpu.make_async_copy(wq_hbm.at[:, pl.ds(off, GW)], wq_v.at[h], swq.at[h])

    wo_copy = pltpu.make_async_copy(wo_hbm, wo_v, sw.at[0])
    w1_copy = pltpu.make_async_copy(w1_hbm, w1_v, sw.at[1])
    w2_copy = pltpu.make_async_copy(w2_hbm, w2_v, sw.at[2])

    wq_copy(0).start()
    for g in range(LOOK):
        for c in stream_copies(g, a_slot(g, g), g % NBUF) + res_copies(g, g % NBUF):
            c.start()
    for h in range(1, HKV):
        wq_copy(h).start()
    wo_copy.start()

    row = lax.broadcasted_iota(jnp.int32, (8, DH), 0)

    def attn_pass(p, x):
        xr = jnp.broadcast_to(_layernorm(x).astype(bf16), (8, D))

        def head_body(h, z):
            if p == 0:
                wq_copy(h).wait()
            y = jnp.dot(xr, wq_v[h], preferred_element_type=f32)
            qf = jnp.zeros((8, DH), f32)
            for r in range(REP):
                qf = jnp.where(row == r, y[:, r * DH:(r + 1) * DH], qf)
            q = qf.astype(bf16)

            def step(c, carry):
                m, l, acc = carry
                t = h * NSTEP + c
                g = p * T + t
                gn = g + LOOK
                sem_n = gn % NBUF
                if p == 0:
                    @pl.when(gn < T)
                    def _():
                        for cp in (stream_copies(gn, a_slot(gn, gn), sem_n)
                                   + res_copies(gn, sem_n)):
                            cp.start()

                    @pl.when(gn == T)
                    def _():
                        w1_copy.start()
                        w2_copy.start()

                    @pl.when(jnp.logical_and(gn >= T, jnp.logical_not(is_extra(gn - T))))
                    def _():
                        for cp in stream_copies(gn - T, sem_n, sem_n):
                            cp.start()
                else:
                    @pl.when(jnp.logical_and(gn < 2 * T, jnp.logical_not(is_extra(gn - T))))
                    def _():
                        for cp in stream_copies(gn - T, sem_n, sem_n):
                            cp.start()

                sem = g % NBUF
                slot = a_slot(g, t)
                if p == 0:
                    for cp in stream_copies(t, slot, sem) + res_copies(t, sem):
                        cp.wait()
                elif NEXTRA == 0:
                    for cp in stream_copies(t, slot, sem):
                        cp.wait()
                else:
                    @pl.when(jnp.logical_not(is_extra(t)))
                    def _():
                        for cp in stream_copies(t, slot, sem):
                            cp.wait()

                sa = lax.dot_general(q, kbuf[slot], _NT, preferred_element_type=f32) * scale
                sb = lax.dot_general(q, kres[t], _NT, preferred_element_type=f32) * scale
                m_new = jnp.maximum(
                    m,
                    jnp.maximum(jnp.max(sa, axis=1, keepdims=True),
                                jnp.max(sb, axis=1, keepdims=True)))
                alpha = jnp.exp(m - m_new)
                pa = jnp.exp(sa - m_new)
                pb = jnp.exp(sb - m_new)
                l = (alpha * l + jnp.sum(pa, axis=1, keepdims=True)
                     + jnp.sum(pb, axis=1, keepdims=True))
                acc = (alpha * acc
                       + jnp.dot(pa.astype(bf16), vbuf[slot], preferred_element_type=f32)
                       + jnp.dot(pb.astype(bf16), vres[t], preferred_element_type=f32))
                return m_new, l, acc

            init = (jnp.full((8, 1), -jnp.inf, f32), jnp.zeros((8, 1), f32),
                    jnp.zeros((8, DH), f32))
            m, l, acc = lax.fori_loop(0, NSTEP, step, init)
            oh = acc / l
            opart = jnp.concatenate(
                [jnp.where(row == r, oh, 0.0).astype(bf16) for r in range(REP)], axis=1)
            if p == 0:
                @pl.when(h == 0)
                def _():
                    wo_copy.wait()
            wo_h = wo_v[pl.ds(pl.multiple_of(h * GW, GW), GW), :]
            return z + jnp.dot(opart, wo_h, preferred_element_type=f32)

        z = lax.fori_loop(0, HKV, head_body, jnp.zeros((8, D), f32))
        return jnp.sum(z, axis=0, keepdims=True)

    def mlp(x):
        xr = jnp.broadcast_to(_layernorm(x).astype(bf16), (8, D))
        b1f = b1_ref[...].astype(f32)
        bias = jnp.concatenate([b1f[j:j + 1, :] for j in range(F // 128)], axis=1)
        h = jnp.dot(xr, w1_v[...], preferred_element_type=f32) + bias
        sp = jnp.log1p(jnp.exp(-jnp.abs(h))) + jnp.where(h > 0, h, jnp.zeros_like(h))
        act = h * jnp.tanh(sp)
        y = jnp.dot(act.astype(bf16), w2_v[...], preferred_element_type=f32)
        return y[0:1, :]

    x = x_ref[...].astype(f32)
    x = x + attn_pass(0, x)
    w1_copy.wait()
    w2_copy.wait()
    x = x + mlp(x)
    x = x + attn_pass(1, x)
    x = x + mlp(x)
    o_ref[...] = x.astype(o_ref.dtype)


@jax.jit
def pallas_interleave_layers__gqa_block_cached__dense_activation_mish__decode_kernel(
    A_x: jax.Array,
    A_k_cache: jax.Array,
    A_v_cache: jax.Array,
    A_wq: jax.Array,
    A_wo: jax.Array,
    B_x: jax.Array,
    B_w1: jax.Array,
    B_b1: jax.Array,
    B_w2: jax.Array,
):
    bf16 = jnp.bfloat16
    x2 = A_x.reshape(1, D)
    k2 = A_k_cache.reshape(HKV * SK, DH)
    v2 = A_v_cache.reshape(HKV * SK, DH)
    b1 = B_b1.reshape(F // 128, 128)

    vmem = pl.BlockSpec(memory_space=pltpu.VMEM)
    hbm = pl.BlockSpec(memory_space=pl.ANY)
    out = pl.pallas_call(
        _kernel,
        out_shape=jax.ShapeDtypeStruct((1, D), A_x.dtype),
        in_specs=[vmem, vmem, hbm, hbm, hbm, hbm, hbm, hbm],
        out_specs=vmem,
        scratch_shapes=[
            pltpu.VMEM((NBUF + NEXTRA, A_ROWS, DH), bf16),
            pltpu.VMEM((NBUF + NEXTRA, A_ROWS, DH), bf16),
            pltpu.VMEM((T, B_ROWS, DH), bf16),
            pltpu.VMEM((T, B_ROWS, DH), bf16),
            pltpu.VMEM((HKV, D, GW), bf16),
            pltpu.VMEM((HQ * DH, D), bf16),
            pltpu.VMEM((D, F), bf16),
            pltpu.VMEM((F, D), bf16),
            pltpu.SemaphoreType.DMA((NBUF,)),
            pltpu.SemaphoreType.DMA((NBUF,)),
            pltpu.SemaphoreType.DMA((NBUF,)),
            pltpu.SemaphoreType.DMA((NBUF,)),
            pltpu.SemaphoreType.DMA((HKV,)),
            pltpu.SemaphoreType.DMA((3,)),
        ],
        compiler_params=pltpu.CompilerParams(vmem_limit_bytes=VMEM_LIMIT),
    )(x2, b1, k2, v2, A_wq, A_wo, B_w1, B_w2)
    return out.reshape(1, 1, D)
```

```python
import jax
import jax.numpy as jnp
from jax import lax
import jax.experimental.pallas as pl
import jax.experimental.pallas.tpu as pltpu

D = 512
HQ = 32
HKV = 8
SK = 65536
DH = 128
F = 1792
REP = HQ // HKV
GW = REP * DH
EPS = 1e-5

A_ROWS = 1152
B_ROWS = 896
CHUNK = A_ROWS + B_ROWS
NSTEP = SK // CHUNK
T = HKV * NSTEP
NBUF = 4
NEXTRA = 3
EXTRA_PERIOD = 64
EXTRA_PHASE = 40
LOOK = NBUF - 1
VMEM_LIMIT = 128 * 1024 * 1024

_NT = (((1,), (1,)), ((), ()))


def _layernorm(x):
    m = jnp.mean(x, axis=-1, keepdims=True)
    xc = x - m
    v = jnp.mean(xc * xc, axis=-1, keepdims=True)
    return xc / jnp.sqrt(v + EPS)


def _kernel(x_hbm, b1_hbm, k_hbm, v_hbm, wq_hbm, wo_hbm, w1_hbm, w2_hbm, o_ref,
            kbuf, vbuf, kres, vres, wq_v, wo_v, w1_v, w2_v, x_ref, b1_ref,
            sk, sv, srk, srv, swq, sw):
    f32 = jnp.float32
    bf16 = jnp.bfloat16
    scale = DH ** -0.5

    def is_extra(t):
        return jnp.logical_and(t % EXTRA_PERIOD == EXTRA_PHASE, t < NEXTRA * EXTRA_PERIOD)

    def a_slot(g, t):
        return jnp.where(is_extra(t), NBUF + t // EXTRA_PERIOD, g % NBUF)

    def stream_copies(t, slot, sem):
        off = pl.multiple_of(t * CHUNK, 128)
        return (
            pltpu.make_async_copy(k_hbm.at[pl.ds(off, A_ROWS)], kbuf.at[slot], sk.at[sem]),
            pltpu.make_async_copy(v_hbm.at[pl.ds(off, A_ROWS)], vbuf.at[slot], sv.at[sem]),
        )

    def res_copies(t, sem):
        off = pl.multiple_of(t * CHUNK + A_ROWS, 128)
        return (
            pltpu.make_async_copy(k_hbm.at[pl.ds(off, B_ROWS)], kres.at[t], srk.at[sem]),
            pltpu.make_async_copy(v_hbm.at[pl.ds(off, B_ROWS)], vres.at[t], srv.at[sem]),
        )

    def wq_copy(h):
        off = h * GW if isinstance(h, int) else pl.multiple_of(h * GW, GW)
        return pltpu.make_async_copy(wq_hbm.at[:, pl.ds(off, GW)], wq_v.at[h], swq.at[h])

    wo_copy = pltpu.make_async_copy(wo_hbm, wo_v, sw.at[0])
    w1_copy = pltpu.make_async_copy(w1_hbm, w1_v, sw.at[1])
    w2_copy = pltpu.make_async_copy(w2_hbm, w2_v, sw.at[2])
    x_copy = pltpu.make_async_copy(x_hbm, x_ref, sw.at[3])
    b1_copy = pltpu.make_async_copy(b1_hbm, b1_ref, sw.at[4])

    wq_copy(0).start()
    x_copy.start()
    for g in range(LOOK):
        for c in stream_copies(g, a_slot(g, g), g % NBUF) + res_copies(g, g % NBUF):
            c.start()
    for h in range(1, HKV):
        wq_copy(h).start()
    wo_copy.start()
    b1_copy.start()

    row = lax.broadcasted_iota(jnp.int32, (8, DH), 0)

    def attn_pass(p, x):
        xr = jnp.broadcast_to(_layernorm(x).astype(bf16), (8, D))

        def head_body(h, z):
            if p == 0:
                wq_copy(h).wait()
            y = jnp.dot(xr, wq_v[h], preferred_element_type=f32)
            qf = jnp.zeros((8, DH), f32)
            for r in range(REP):
                qf = jnp.where(row == r, y[:, r * DH:(r + 1) * DH], qf)
            q = qf.astype(bf16)

            def step(c, carry):
                m, l, acc = carry
                t = h * NSTEP + c
                g = p * T + t
                gn = g + LOOK
                sem_n = gn % NBUF
                if p == 0:
                    @pl.when(gn < T)
                    def _():
                        for cp in (stream_copies(gn, a_slot(gn, gn), sem_n)
                                   + res_copies(gn, sem_n)):
                            cp.start()

                    @pl.when(gn == T)
                    def _():
                        w1_copy.start()
                        w2_copy.start()

                    @pl.when(jnp.logical_and(gn >= T, jnp.logical_not(is_extra(gn - T))))
                    def _():
                        for cp in stream_copies(gn - T, sem_n, sem_n):
                            cp.start()
                else:
                    @pl.when(jnp.logical_and(gn < 2 * T, jnp.logical_not(is_extra(gn - T))))
                    def _():
                        for cp in stream_copies(gn - T, sem_n, sem_n):
                            cp.start()

                sem = g % NBUF
                slot = a_slot(g, t)
                if p == 0:
                    for cp in stream_copies(t, slot, sem) + res_copies(t, sem):
                        cp.wait()
                else:
                    @pl.when(jnp.logical_not(is_extra(t)))
                    def _():
                        for cp in stream_copies(t, slot, sem):
                            cp.wait()

                sa = lax.dot_general(q, kbuf[slot], _NT, preferred_element_type=f32) * scale
                sb = lax.dot_general(q, kres[t], _NT, preferred_element_type=f32) * scale
                m_new = jnp.maximum(
                    m,
                    jnp.maximum(jnp.max(sa, axis=1, keepdims=True),
                                jnp.max(sb, axis=1, keepdims=True)))
                alpha = jnp.exp(m - m_new)
                pa = jnp.exp(sa - m_new)
                pb = jnp.exp(sb - m_new)
                l = (alpha * l + jnp.sum(pa, axis=1, keepdims=True)
                     + jnp.sum(pb, axis=1, keepdims=True))
                acc = (alpha * acc
                       + jnp.dot(pa.astype(bf16), vbuf[slot], preferred_element_type=f32)
                       + jnp.dot(pb.astype(bf16), vres[t], preferred_element_type=f32))
                return m_new, l, acc

            init = (jnp.full((8, 1), -jnp.inf, f32), jnp.zeros((8, 1), f32),
                    jnp.zeros((8, DH), f32))
            m, l, acc = lax.fori_loop(0, NSTEP, step, init)
            oh = acc / l
            opart = jnp.concatenate(
                [jnp.where(row == r, oh, 0.0).astype(bf16) for r in range(REP)], axis=1)
            if p == 0:
                @pl.when(h == 0)
                def _():
                    wo_copy.wait()
            wo_h = wo_v[pl.ds(pl.multiple_of(h * GW, GW), GW), :]
            return z + jnp.dot(opart, wo_h, preferred_element_type=f32)

        z = lax.fori_loop(0, HKV, head_body, jnp.zeros((8, D), f32))
        return jnp.sum(z, axis=0, keepdims=True)

    def mlp(x):
        xr = jnp.broadcast_to(_layernorm(x).astype(bf16), (8, D))
        b1f = b1_ref[...].astype(f32)
        bias = jnp.concatenate([b1f[j:j + 1, :] for j in range(F // 128)], axis=1)
        h = jnp.dot(xr, w1_v[...], preferred_element_type=f32) + bias
        sp = jnp.log1p(jnp.exp(-jnp.abs(h))) + jnp.where(h > 0, h, jnp.zeros_like(h))
        act = h * jnp.tanh(sp)
        y = jnp.dot(act.astype(bf16), w2_v[...], preferred_element_type=f32)
        return y[0:1, :]

    x_copy.wait()
    x = x_ref[...].astype(f32)
    x = x + attn_pass(0, x)
    b1_copy.wait()
    w1_copy.wait()
    w2_copy.wait()
    x = x + mlp(x)
    x = x + attn_pass(1, x)
    x = x + mlp(x)
    o_ref[...] = x.astype(o_ref.dtype)


@jax.jit
def pallas_interleave_layers__gqa_block_cached__dense_activation_mish__decode_kernel(
    A_x: jax.Array,
    A_k_cache: jax.Array,
    A_v_cache: jax.Array,
    A_wq: jax.Array,
    A_wo: jax.Array,
    B_x: jax.Array,
    B_w1: jax.Array,
    B_b1: jax.Array,
    B_w2: jax.Array,
):
    bf16 = jnp.bfloat16
    x2 = A_x.reshape(1, D)
    k2 = A_k_cache.reshape(HKV * SK, DH)
    v2 = A_v_cache.reshape(HKV * SK, DH)
    b1 = B_b1.reshape(F // 128, 128)

    vmem = pl.BlockSpec(memory_space=pltpu.VMEM)
    hbm = pl.BlockSpec(memory_space=pl.ANY)
    out = pl.pallas_call(
        _kernel,
        out_shape=jax.ShapeDtypeStruct((1, D), A_x.dtype),
        in_specs=[hbm] * 8,
        out_specs=vmem,
        scratch_shapes=[
            pltpu.VMEM((NBUF + NEXTRA, A_ROWS, DH), bf16),
            pltpu.VMEM((NBUF + NEXTRA, A_ROWS, DH), bf16),
            pltpu.VMEM((T, B_ROWS, DH), bf16),
            pltpu.VMEM((T, B_ROWS, DH), bf16),
            pltpu.VMEM((HKV, D, GW), bf16),
            pltpu.VMEM((HQ * DH, D), bf16),
            pltpu.VMEM((D, F), bf16),
            pltpu.VMEM((F, D), bf16),
            pltpu.VMEM((1, D), bf16),
            pltpu.VMEM((F // 128, 128), bf16),
            pltpu.SemaphoreType.DMA((NBUF,)),
            pltpu.SemaphoreType.DMA((NBUF,)),
            pltpu.SemaphoreType.DMA((NBUF,)),
            pltpu.SemaphoreType.DMA((NBUF,)),
            pltpu.SemaphoreType.DMA((HKV,)),
            pltpu.SemaphoreType.DMA((5,)),
        ],
        compiler_params=pltpu.CompilerParams(vmem_limit_bytes=VMEM_LIMIT),
    )(x2, b1, k2, v2, A_wq, A_wo, B_w1, B_w2)
    return out.reshape(1, 1, D)
```
